```python
import os as _os
_os.environ.setdefault("JAX_PLATFORMS", "cpu")
import jax
import jax.numpy as jnp

def _softmax(x, axis=-1):
    return jax.nn.softmax(x, axis=axis)
def _gelu(x):
    return jax.nn.gelu(x, approximate=True)
def _silu(x):
    return jax.nn.silu(x)
def _sigmoid(x):
    return jax.nn.sigmoid(x)
def _layernorm(x, axis=-1, eps=1e-5):
    m = jnp.mean(x, axis=axis, keepdims=True)
    v = jnp.var(x, axis=axis, keepdims=True)
    return (x - m) / jnp.sqrt(v + eps)
def _scatter_add(tgt, idx, src, axis=0):
    return tgt.at[idx].add(src)
def _segment_sum(src, seg, n):
    return jax.ops.segment_sum(src, seg, n)
class _Rng:
    def __init__(self, key):
        self._k = key
    def _next(self):
        self._k, sub = jax.random.split(self._k)
        return sub
    def normal(self, shape):
        return jax.random.normal(self._next(), shape, dtype=jnp.bfloat16)
    def randint(self, lo, hi, shape):
        return jax.random.randint(self._next(), shape, lo, hi, dtype=jnp.int32)
    def uniform(self, shape, lo=0.0, hi=1.0):
        return jax.random.uniform(self._next(), shape, jnp.bfloat16, lo, hi)
    def permutation(self, n):
        return jax.random.permutation(self._next(), n)


kernel_name = 'concat_heads__spectral_gfnet__sliding_block__prompt'

def setup_inputs():
    _rng = _Rng(jax.random.key(int.from_bytes(__import__("os").urandom(4), "little")))
    _w = (lambda a: (lambda t: t.astype(jnp.bfloat16) if jnp.issubdtype(t.dtype, jnp.floating) else t)(jnp.asarray(a)))
    def _A_setup():
        B, S, D = 1, 2048, 640
        Df = D // 2 + 1
        return {
            "x": _w((lambda *s: _rng.normal(s) * 0.05)(B, S, D)),
            "w_r": _w((lambda *s: _rng.normal(s) * 0.4)(S, Df) * 0.02),
            "w_i": _w((lambda *s: _rng.normal(s) * 0.4)(S, Df) * 0.02),
        }
    _A_in = _A_setup()

    def _B_setup():
        B, S, D = 1, 2048, 640
        return {
            "x": _w((lambda *s: _rng.normal(s) * 0.2)(B, S, D)),
            "wqkv": _w((lambda *s: _rng.normal(s) * 0.2)(D, 3 * D)),
            "wo": _w((lambda *s: _rng.normal(s) * 0.05)(D, D)),
        }
    _B_in = _B_setup()

    return {
        "A_x": _A_in["x"],
        "A_w_r": _A_in["w_r"],
        "A_w_i": _A_in["w_i"],
        "B_x": _B_in["x"],
        "B_wqkv": _B_in["wqkv"],
        "B_wo": _B_in["wo"],
    }

def reference(A_x, A_w_r, A_w_i, B_x, B_wqkv, B_wo):
    def _A_ref(x, w_r, w_i):
        B, S, D = x.shape
        X = (lambda x, axes=(-2,-1): jnp.fft.rfft2(x.astype(jnp.float32), axes=axes))(x, axes=(-2, -1))
        W = w_r + 1j * w_i
        X = X * W
        y = (lambda x, s, axes=(-2,-1): jnp.fft.irfft2(x, s=s, axes=axes).astype(jnp.bfloat16))(X, (S, D), axes=(-2, -1))
        return y

    def _B_ref(x, wqkv, wo):
        B, S, D = x.shape
        H = 32; Dh = D // H; W = 256
        qkv = (lambda x, *d: x.transpose(*d))((x @ wqkv).reshape(B, S, 3, H, Dh), 2, 0, 3, 1, 4)
        q, k, v = qkv[0], qkv[1], qkv[2]
        scores = jnp.einsum("bhqd,bhkd->bhqk", q, k) * (Dh ** -0.5)
        idx = jnp.arange(S)
        mask = (idx[:, None] - idx[None, :] >= 0) & (idx[:, None] - idx[None, :] < W)
        scores = jnp.where(mask[None, None], scores, -1e9)
        p = _softmax(scores, axis=-1)
        o = jnp.einsum("bhqk,bhkd->bhqd", p, v)
        return (lambda x, *d: x.transpose(*d))(o, 0, 2, 1, 3).reshape(B, S, D) @ wo

    a = _A_ref(A_x, A_w_r, A_w_i)
    b = _B_ref(B_x, B_wqkv, B_wo)
    return jnp.concatenate([a, b], axis=-1)
```

```python
import math

import numpy as np
import jax
import jax.numpy as jnp
from jax import lax
import jax.experimental.pallas as pl
import jax.experimental.pallas.tpu as pltpu

S = 2048
D = 640
DF = D // 2 + 1
FP = 384
H = 32
DH = 20
WIN = 256
HPG = 6
NG = 6
QW = NG * 128
N1 = 16
N2 = 128
BQ = 128
NQB = S // BQ
KSPAN = 3 * BQ
KPAD = 2 * BQ
NEG = -1e30

_F32 = jnp.float32
_BF16 = jnp.bfloat16


def _tables():
    d = np.arange(D, dtype=np.float64)
    f = np.arange(DF, dtype=np.float64)
    ang = 2.0 * np.pi * np.outer(d, f) / D
    fd = np.zeros((D, 2 * FP), np.float64)
    fd[:, :DF] = np.cos(ang)
    fd[:, FP:FP + DF] = -np.sin(ang)
    c = np.full((DF,), 2.0)
    c[0] = 1.0
    c[-1] = 1.0
    g = np.zeros((2 * FP, D), np.float64)
    scale = 1.0 / (D * S)
    g[:DF, :] = (c[:, None] * np.cos(ang.T)) * scale
    g[FP:FP + DF, :] = (-c[:, None] * np.sin(ang.T)) * scale
    k1 = np.arange(N1)[:, None, None]
    k2 = np.arange(N2)[None, :, None]
    n2 = np.arange(N2)[None, None, :]
    a = 2.0 * np.pi * ((n2 * (k1 + N1 * k2)) % S) / S
    tr = np.cos(a)
    ti = -np.sin(a)
    tf = np.concatenate([tr, ti], axis=1)
    tb = np.concatenate([tr.transpose(0, 2, 1), ti.transpose(0, 2, 1)], axis=1)
    e = np.zeros((128, 128), np.float64)
    for h in range(HPG):
        e[HPG * DH + h, h * DH:(h + 1) * DH] = 1.0
    return (jnp.asarray(fd, _BF16), jnp.asarray(g, _BF16),
            jnp.asarray(tf, _BF16), jnp.asarray(tb, _BF16),
            jnp.asarray(e, _BF16))


def _cmul_const(xr, xi, wr, wi):
    eps = 1e-12
    if abs(wi) < eps:
        if abs(wr - 1.0) < eps:
            return xr, xi
        if abs(wr + 1.0) < eps:
            return -xr, -xi
    if abs(wr) < eps:
        if abs(wi - 1.0) < eps:
            return -xi, xr
        if abs(wi + 1.0) < eps:
            return xi, -xr
    if abs(abs(wr) - abs(wi)) < eps:
        s = abs(wr)
        a = xr * s
        b = xi * s
        sr = 1.0 if wr > 0 else -1.0
        si = 1.0 if wi > 0 else -1.0
        re = (a - b) if (sr > 0 and si > 0) else (a + b) if (sr > 0) else (
            (-a - b) if si > 0 else (b - a))
        im = (a + b) if (si > 0 and sr > 0) else (b - a) if (sr > 0) else (
            (a - b) if si > 0 else (-a - b))
        return re, im
    return xr * wr - xi * wi, xr * wi + xi * wr


def _fft_list(xs, sign):
    n = len(xs)
    if n == 1:
        return xs
    ev = _fft_list(xs[0::2], sign)
    od = _fft_list(xs[1::2], sign)
    out = [None] * n
    for k in range(n // 2):
        ang = sign * 2.0 * math.pi * k / n
        tr, ti = _cmul_const(od[k][0], od[k][1], math.cos(ang), math.sin(ang))
        out[k] = (ev[k][0] + tr, ev[k][1] + ti)
        out[k + n // 2] = (ev[k][0] - tr, ev[k][1] - ti)
    return out


def _dot(a, b):
    return jnp.dot(a, b, preferred_element_type=_F32)


def _kernel(xa_h, wr_h, wi_h, xb_h, wqkv_h, wo_h, fd_h, g_h, tf_h, tb_h, e_h,
            out_h,
            xa_v, wr_v, wi_v, xb_v, wqkv_v, wo_v, fd_v, g_v, tf_v, tb_v, e_v,
            wrf, wif, zs, q_s, kt_s, v_s, o_s, ya_buf, yb_buf,
            in_sems, oa_sems, ob_sems):
    copies = [
        pltpu.make_async_copy(xa_h, xa_v, in_sems.at[0]),
        pltpu.make_async_copy(fd_h, fd_v, in_sems.at[1]),
        pltpu.make_async_copy(xb_h, xb_v, in_sems.at[2]),
        pltpu.make_async_copy(wqkv_h, wqkv_v, in_sems.at[3]),
        pltpu.make_async_copy(tf_h, tf_v, in_sems.at[4]),
        pltpu.make_async_copy(wr_h, wr_v, in_sems.at[5]),
        pltpu.make_async_copy(wi_h, wi_v, in_sems.at[6]),
        pltpu.make_async_copy(tb_h, tb_v, in_sems.at[7]),
        pltpu.make_async_copy(g_h, g_v, in_sems.at[8]),
        pltpu.make_async_copy(e_h, e_v, in_sems.at[9]),
        pltpu.make_async_copy(wo_h, wo_v, in_sems.at[10]),
    ]
    for c in copies:
        c.start()

    kt_s[:, 0:KPAD] = jnp.zeros((QW, KPAD), _BF16)
    v_s[0:KPAD, :] = jnp.zeros((KPAD, QW), _BF16)

    copies[0].wait()
    copies[1].wait()
    RC = 256

    def a_dft(c, carry):
        r0 = pl.multiple_of(c * RC, RC)
        zs[pl.ds(r0, RC), :] = _dot(xa_v[pl.ds(r0, RC), :], fd_v[...])
        return carry

    lax.fori_loop(0, S // RC, a_dft, 0)

    def slab_fft(sign):
        def body(r, carry):
            r0 = pl.multiple_of(r * 8, 8)
            for t in range(FP // 128):
                xs = []
                for n1 in range(N1):
                    rows = pl.ds(n1 * N2 + r0, 8)
                    xs.append((zs[rows, pl.ds(t * 128, 128)],
                               zs[rows, pl.ds(FP + t * 128, 128)]))
                ys = _fft_list(xs, sign)
                for k1 in range(N1):
                    rows = pl.ds(k1 * N2 + r0, 8)
                    zs[rows, pl.ds(t * 128, 128)] = ys[k1][0]
                    zs[rows, pl.ds(FP + t * 128, 128)] = ys[k1][1]
            return carry

        lax.fori_loop(0, N2 // 8, body, 0)

    slab_fft(-1.0)

    copies[4].wait()
    copies[5].wait()
    copies[6].wait()
    copies[7].wait()

    def w_cvt(c, carry):
        r0 = pl.multiple_of(c * RC, RC)
        for src, dst in ((wr_v, wrf), (wi_v, wif)):
            dst[0, pl.ds(r0, RC), :] = src[pl.ds(r0, RC), 0:128].astype(_F32)
            dst[1, pl.ds(r0, RC), :] = src[pl.ds(r0, RC), 128:256].astype(_F32)
            dst[2, pl.ds(r0, RC), :] = jnp.zeros((RC, 128), _F32)
            dst[2, pl.ds(r0, RC), 0:DF - 256] = src[pl.ds(r0, RC), 256:DF].astype(_F32)
        return carry

    lax.fori_loop(0, S // RC, w_cvt, 0)

    def a_mid(k1, carry):
        r0 = pl.multiple_of(k1 * N2, N2)
        a = zs[pl.ds(r0, N2), :].astype(_BF16)
        pq = _dot(tf_v[k1], a)
        xr = pq[:N2, :FP] - pq[N2:, FP:]
        xi = pq[:N2, FP:] + pq[N2:, :FP]
        wr = jnp.concatenate(
            [wrf[t, pl.ds(k1, N2, stride=N1), :] for t in range(3)], axis=1)
        wi = jnp.concatenate(
            [wif[t, pl.ds(k1, N2, stride=N1), :] for t in range(3)], axis=1)
        yr = xr * wr - xi * wi
        yi = xr * wi + xi * wr
        y = jnp.concatenate([yr, yi], axis=1).astype(_BF16)
        pq = _dot(tb_v[k1], y)
        zs[pl.ds(r0, N2), pl.ds(0, FP)] = pq[:N2, :FP] + pq[N2:, FP:]
        zs[pl.ds(r0, N2), pl.ds(FP, FP)] = pq[:N2, FP:] - pq[N2:, :FP]
        return carry

    lax.fori_loop(0, N1, a_mid, 0)

    slab_fft(1.0)

    copies[8].wait()

    def a_out_copy(c):
        r0 = pl.multiple_of(c * RC, RC)
        return pltpu.make_async_copy(
            ya_buf.at[pl.ds(r0, RC), :],
            out_h.at[pl.ds(r0, RC), pl.ds(0, D)],
            oa_sems.at[c])

    def a_idft(c, carry):
        r0 = pl.multiple_of(c * RC, RC)
        z = zs[pl.ds(r0, RC), :].astype(_BF16)
        ya_buf[pl.ds(r0, RC), :] = _dot(z, g_v[...]).astype(_BF16)
        a_out_copy(c).start()
        return carry

    lax.fori_loop(0, S // RC, a_idft, 0)

    copies[2].wait()
    copies[3].wait()

    lane = lax.broadcasted_iota(jnp.int32, (1, 128), 1)

    def b_qkv(c, carry):
        r0 = pl.multiple_of(c * RC, RC)
        x = xb_v[pl.ds(r0, RC), :]
        q_s[pl.ds(r0, RC), :] = _dot(x, wqkv_v[:, 0:QW]).astype(_BF16)
        k = _dot(x, wqkv_v[:, QW:2 * QW])
        kt_s[:, pl.ds(KPAD + r0, RC)] = k.T.astype(_BF16)
        v = _dot(x, wqkv_v[:, 2 * QW:3 * QW])
        lane_q = lax.broadcasted_iota(jnp.int32, (RC, QW), 1) % 128
        v = jnp.where(lane_q >= HPG * DH, 1.0, v)
        v_s[pl.ds(KPAD + r0, RC), :] = v.astype(_BF16)
        return carry

    lax.fori_loop(0, S // RC, b_qkv, 0)

    copies[9].wait()
    cexp = (DH ** -0.5) * math.log2(math.e)

    def b_attn(i, carry):
        r0 = pl.multiple_of(i * BQ, BQ)
        row = lax.broadcasted_iota(jnp.int32, (BQ, KSPAN), 0)
        col = lax.broadcasted_iota(jnp.int32, (BQ, KSPAN), 1)
        valid = (col > row) & (col <= row + WIN) & (col + (i - 2) * BQ >= 0)
        bias = jnp.where(valid, 0.0, NEG).astype(_F32)
        for g in range(NG):
            nh = min(HPG, H - g * HPG)
            qb = q_s[pl.ds(r0, BQ), pl.ds(g * 128, 128)]
            masks = [((lane >= h * DH) & (lane < (h + 1) * DH)) for h in range(nh)]
            qm = jnp.concatenate(
                [jnp.where(masks[h], qb, jnp.zeros_like(qb)) for h in range(nh)],
                axis=0)
            kt = kt_s[pl.ds(g * 128, 128), pl.ds(r0, KSPAN)]
            s = _dot(qm, kt).reshape(nh, BQ, KSPAN) + bias[None]
            m = jnp.max(s, axis=-1, keepdims=True)
            p = jnp.exp2((s - m) * cexp).astype(_BF16)
            vg = v_s[pl.ds(r0, KSPAN), pl.ds(g * 128, 128)]
            oh = _dot(p.reshape(nh * BQ, KSPAN), vg).reshape(nh, BQ, 128)
            o = jnp.zeros((BQ, 128), _F32)
            for h in range(nh):
                mh = masks[h] | (lane == HPG * DH + h)
                o = jnp.where(mh, oh[h], o)
            dvalid = (lane >= HPG * DH) & (lane < HPG * DH + nh)
            r = jnp.where(dvalid, 1.0 / jnp.where(dvalid, o, 1.0), 0.0)
            rh = r.astype(_BF16)
            rl = (r - rh.astype(_F32)).astype(_BF16)
            rb = _dot(rh, e_v[...]) + _dot(rl, e_v[...])
            o_s[pl.ds(r0, BQ), pl.ds(g * 128, 128)] = (o * rb).astype(_BF16)
        return carry

    lax.fori_loop(0, NQB, b_attn, 0)

    copies[10].wait()

    def b_out_copy(c):
        r0 = pl.multiple_of(c * RC, RC)
        return pltpu.make_async_copy(
            yb_buf.at[pl.ds(r0, RC), :],
            out_h.at[pl.ds(r0, RC), pl.ds(D, D)],
            ob_sems.at[c])

    def b_proj(c, carry):
        r0 = pl.multiple_of(c * RC, RC)
        yb_buf[pl.ds(r0, RC), :] = _dot(o_s[pl.ds(r0, RC), :], wo_v[...]).astype(_BF16)
        b_out_copy(c).start()
        return carry

    lax.fori_loop(0, S // RC, b_proj, 0)

    for c in range(S // RC):
        a_out_copy(c).wait()
        b_out_copy(c).wait()


def _pad_heads_cols(w):
    w = jnp.pad(w, ((0, 0), (0, NG * HPG * DH - D)))
    w = w.reshape(D, NG, HPG * DH)
    w = jnp.pad(w, ((0, 0), (0, 0), (0, 128 - HPG * DH)))
    return w.reshape(D, QW)


@jax.jit
def pallas_concat_heads__spectral_gfnet__sliding_block__prompt_kernel(
    A_x: jax.Array,
    A_w_r: jax.Array,
    A_w_i: jax.Array,
    B_x: jax.Array,
    B_wqkv: jax.Array,
    B_wo: jax.Array,
):
    fd, g, tf, tb, e = _tables()
    xa = A_x.reshape(S, D)
    xb = B_x.reshape(S, D)
    wqkv = jnp.concatenate(
        [_pad_heads_cols(B_wqkv[:, j * D:(j + 1) * D]) for j in range(3)], axis=1)
    wo = _pad_heads_cols(B_wo.T).T

    any_spec = pl.BlockSpec(memory_space=pl.ANY)
    nrc = S // 256
    out = pl.pallas_call(
        _kernel,
        out_shape=jax.ShapeDtypeStruct((S, 2 * D), _BF16),
        in_specs=[any_spec] * 11,
        out_specs=any_spec,
        scratch_shapes=[
            pltpu.VMEM((S, D), _BF16),
            pltpu.VMEM((S, DF), _BF16),
            pltpu.VMEM((S, DF), _BF16),
            pltpu.VMEM((S, D), _BF16),
            pltpu.VMEM((D, 3 * QW), _BF16),
            pltpu.VMEM((QW, D), _BF16),
            pltpu.VMEM((D, 2 * FP), _BF16),
            pltpu.VMEM((2 * FP, D), _BF16),
            pltpu.VMEM((N1, 2 * N2, N2), _BF16),
            pltpu.VMEM((N1, 2 * N2, N2), _BF16),
            pltpu.VMEM((128, 128), _BF16),
            pltpu.VMEM((3, S, 128), _F32),
            pltpu.VMEM((3, S, 128), _F32),
            pltpu.VMEM((S, 2 * FP), _F32),
            pltpu.VMEM((S, QW), _BF16),
            pltpu.VMEM((QW, S + KPAD), _BF16),
            pltpu.VMEM((S + KPAD, QW), _BF16),
            pltpu.VMEM((S, QW), _BF16),
            pltpu.VMEM((S, D), _BF16),
            pltpu.VMEM((S, D), _BF16),
            pltpu.SemaphoreType.DMA((11,)),
            pltpu.SemaphoreType.DMA((nrc,)),
            pltpu.SemaphoreType.DMA((nrc,)),
        ],
        compiler_params=pltpu.CompilerParams(
            vmem_limit_bytes=100 * 1024 * 1024),
    )(xa, A_w_r, A_w_i, xb, wqkv, wo, fd, g, tf, tb, e)
    return out.reshape(1, S, 2 * D)
```

```python
import functools
import math

import numpy as np
import jax
import jax.numpy as jnp
from jax import lax
import jax.experimental.pallas as pl
import jax.experimental.pallas.tpu as pltpu

S = 2048
D = 640
DF = D // 2 + 1
FP = 384
H = 32
DH = 20
WIN = 256
HPG = 6
NG = 6
QW = NG * 128
N1 = 16
N2 = 128
SB = 64
NT = WIN // SB + 1
GW = HPG * SB
RING = 8
RC = 256
NRC = S // RC
WTR = 360
NEG = -1e30

_F32 = jnp.float32
_BF16 = jnp.bfloat16

_C1 = math.cos(2.0 * math.pi / 5.0)
_C2 = math.cos(4.0 * math.pi / 5.0)
_S1 = math.sin(2.0 * math.pi / 5.0)
_S2 = math.sin(4.0 * math.pi / 5.0)


def _tables():
    b = np.arange(128, dtype=np.float64)[:, None]
    f2 = np.arange(64, dtype=np.float64)[None, :]

    def ang(f1, n=64):
        f = f1 + 5.0 * np.arange(n, dtype=np.float64)[None, :]
        return 2.0 * np.pi * ((b * f) % D) / D

    scale = 1.0 / (D * S)
    fm = np.zeros((2, 256, 256), np.float64)
    im = np.zeros((2, 256, 256), np.float64)
    for p, (fa, fb) in enumerate(((1, 4), (2, 3))):
        ta, tb_ = ang(fa), ang(fb)
        fm[p, :128, 0:64] = np.cos(ta)
        fm[p, 128:, 0:64] = np.sin(ta)
        fm[p, :128, 64:128] = np.cos(tb_)
        fm[p, 128:, 64:128] = -np.sin(tb_)
        fm[p, :128, 128:192] = -np.sin(ta)
        fm[p, 128:, 128:192] = np.cos(ta)
        fm[p, :128, 192:256] = -np.sin(tb_)
        fm[p, 128:, 192:256] = -np.cos(tb_)
        c = 2.0 * scale
        im[p, 0:64, :128] = c * np.cos(ta).T
        im[p, 128:192, :128] = -c * np.sin(ta).T
        im[p, 0:64, 128:] = c * np.sin(ta).T
        im[p, 128:192, 128:] = c * np.cos(ta).T
        im[p, 64:128, :128] = c * np.cos(tb_).T
        im[p, 192:256, :128] = -c * np.sin(tb_).T
        im[p, 64:128, 128:] = -c * np.sin(tb_).T
        im[p, 192:256, 128:] = -c * np.cos(tb_).T
    t0 = ang(0, 65)
    fm0 = np.zeros((128, 256), np.float64)
    fm0[:, 0:65] = np.cos(t0)
    fm0[:, 128:128 + 65] = -np.sin(t0)
    cf = np.full((65,), 2.0)
    cf[0] = 1.0
    cf[-1] = 1.0
    im0 = np.zeros((256, 128), np.float64)
    im0[0:65, :] = scale * cf[:, None] * np.cos(t0).T
    im0[128:128 + 65, :] = -scale * cf[:, None] * np.sin(t0).T
    k1 = np.arange(N1)[:, None, None]
    k2 = np.arange(N2)[None, :, None]
    n2 = np.arange(N2)[None, None, :]
    a = 2.0 * np.pi * ((n2 * (k1 + N1 * k2)) % S) / S
    tr = np.cos(a)
    ti = -np.sin(a)
    tf = np.concatenate([tr, ti], axis=1)
    tb = np.concatenate([tr.transpose(0, 2, 1), ti.transpose(0, 2, 1)], axis=1)
    c = lambda t: jnp.asarray(t, _BF16)
    return c(fm), c(fm0), c(im), c(im0), c(tf), c(tb)


def _cmul_const(xr, xi, wr, wi):
    eps = 1e-12
    if abs(wi) < eps:
        if abs(wr - 1.0) < eps:
            return xr, xi
        if abs(wr + 1.0) < eps:
            return -xr, -xi
    if abs(wr) < eps:
        if abs(wi - 1.0) < eps:
            return -xi, xr
        if abs(wi + 1.0) < eps:
            return xi, -xr
    if abs(abs(wr) - abs(wi)) < eps:
        s = abs(wr)
        a = xr * s
        b = xi * s
        sr = 1.0 if wr > 0 else -1.0
        si = 1.0 if wi > 0 else -1.0
        re = (a - b) if (sr > 0 and si > 0) else (a + b) if (sr > 0) else (
            (-a - b) if si > 0 else (b - a))
        im = (a + b) if (si > 0 and sr > 0) else (b - a) if (sr > 0) else (
            (a - b) if si > 0 else (-a - b))
        return re, im
    return xr * wr - xi * wi, xr * wi + xi * wr


def _fft_list(xs, sign):
    n = len(xs)
    if n == 1:
        return xs
    ev = _fft_list(xs[0::2], sign)
    od = _fft_list(xs[1::2], sign)
    out = [None] * n
    for k in range(n // 2):
        ang = sign * 2.0 * math.pi * k / n
        tr, ti = _cmul_const(od[k][0], od[k][1], math.cos(ang), math.sin(ang))
        out[k] = (ev[k][0] + tr, ev[k][1] + ti)
        out[k + n // 2] = (ev[k][0] - tr, ev[k][1] - ti)
    return out


def _dot(a, b):
    return jnp.dot(a, b, preferred_element_type=_F32)


def _cat(xs, axis=1):
    return jnp.concatenate(xs, axis=axis)


def _kernel(xa_h, wrt_h, wit_h, xb_h, wqkv_h, wo_h,
            fm_h, fm0_h, im_h, im0_h, tf_h, tb_h,
            out_h,
            wo_v, fm_v, fm0_v, im_v, im0_v, tf_v, tb_v,
            wrf, wif, zs, q_s, kp_s, vp_s, o_acc, o_s, xm_buf, ym_buf,
            ya_buf, yb_buf,
            in_sems, xa_sems, xb_sems, wo_sems, oa_sems, ob_sems):
    lane = lax.broadcasted_iota(jnp.int32, (1, 128), 1)
    masks = [((lane >= h * DH) & (lane < (h + 1) * DH)) for h in range(HPG)]
    cexp = (DH ** -0.5) * math.log2(math.e)

    def loop(n, fn, lo=0):
        def body(i, carry):
            fn(i)
            return carry
        lax.fori_loop(lo, n, body, 0)

    def nheads(g):
        return min(HPG, H - g * HPG)

    cp = {}

    def start(idx, name, src, dst):
        cp[name] = pltpu.make_async_copy(src, dst, in_sems.at[idx])
        cp[name].start()

    def late_copy(name):
        idx, src, dst = {"tf": (5, tf_h, tf_v), "tb": (6, tb_h, tb_v),
                         "im": (7, im_h, im_v), "im0": (8, im0_h, im0_v)}[name]
        return pltpu.make_async_copy(src, dst, in_sems.at[idx])

    def wo_copy(g):
        n = nheads(g) * DH
        return pltpu.make_async_copy(
            wo_h.at[pl.ds(g * HPG * DH, n), :],
            wo_v.at[pl.ds(g * 128, n), :], wo_sems.at[g])

    def fft_rows(r, sign):
        r0 = pl.multiple_of(r * 8, 8)
        for t in range(FP // 128):
            xs = []
            for n1 in range(N1):
                rows = pl.ds(n1 * N2 + r0, 8)
                xs.append((zs[rows, pl.ds(t * 128, 128)],
                           zs[rows, pl.ds(FP + t * 128, 128)]))
            ys = _fft_list(xs, sign)
            for k1 in range(N1):
                rows = pl.ds(k1 * N2 + r0, 8)
                zs[rows, pl.ds(t * 128, 128)] = ys[k1][0]
                zs[rows, pl.ds(FP + t * 128, 128)] = ys[k1][1]

    def early(xa_v, wrt_v, wit_v, xb_v, wqkv_r, wqkv_v, wtf):
        def chunk_copy(src, dst, sems, c):
            r0 = pl.multiple_of(c * RC, RC)
            return pltpu.make_async_copy(
                src.at[pl.ds(r0, RC), :], dst.at[pl.ds(r0, RC), :], sems.at[c])

        start(0, "fm", fm_h, fm_v)
        start(1, "fm0", fm0_h, fm0_v)
        for c in range(NRC):
            chunk_copy(xa_h, xa_v, xa_sems, c).start()

        for g in range(NG):
            n = nheads(g) * DH
            wo_v[g * 128 + n:(g + 1) * 128, :] = jnp.zeros((128 - n, D), _BF16)

        def start_rest():
            start(2, "wqkv", wqkv_h, wqkv_r)
            for c in range(2):
                chunk_copy(xb_h, xb_v, xb_sems, c).start()
            start(3, "wrt", wrt_h, wrt_v)
            start(4, "wit", wit_h, wit_v)
            for c in range(2, NRC):
                chunk_copy(xb_h, xb_v, xb_sems, c).start()
            late_copy("tf").start()
            late_copy("tb").start()
            for g in range(NG):
                wo_copy(g).start()
            late_copy("im").start()
            late_copy("im0").start()

        for b in range(4):
            wtf[b, 320:WTR, :] = jnp.zeros((WTR - 320, 128), _F32)
        q_s[S:S + 4 * SB, :] = jnp.zeros((4 * SB, QW), _BF16)

        def a_dft(c):
            r0 = pl.multiple_of(c * RC, RC)
            rows = pl.ds(r0, RC)
            xs = [xa_v[rows, a * 128:(a + 1) * 128].astype(_F32) for a in range(5)]
            t1 = xs[1] + xs[4]
            t2 = xs[2] + xs[3]
            t3 = xs[1] - xs[4]
            t4 = xs[2] - xs[3]
            a0 = xs[0] + t1 + t2
            a1r = xs[0] + _C1 * t1 + _C2 * t2
            a1i = -(_S1 * t3 + _S2 * t4)
            a2r = xs[0] + _C2 * t1 + _C1 * t2
            a2i = _S1 * t4 - _S2 * t3
            m1 = _dot(_cat([a1r, a1i]).astype(_BF16), fm_v[0])
            m2 = _dot(_cat([a2r, a2i]).astype(_BF16), fm_v[1])
            m0 = _dot(a0.astype(_BF16), fm0_v[...])
            for t, m in enumerate((m1, m2, m0)):
                zs[rows, t * 128:(t + 1) * 128] = m[:, :128]
                zs[rows, FP + t * 128:FP + (t + 1) * 128] = m[:, 128:]

        def w_prep(t, slot):
            c0 = pl.multiple_of(t * 128, 128)
            for b, (src, dst) in enumerate(((wrt_v, wrf), (wit_v, wif))):
                stage = wtf.at[2 * slot + b]
                stage[0:DF, :] = src[:, pl.ds(c0, 128)].astype(_F32)
                fam = lambda f1, n: stage[pl.ds(f1, n, stride=5), :]
                tiles = (
                    _cat([fam(1, 64), fam(4, 64)], axis=0),
                    _cat([fam(2, 64), fam(3, 64)], axis=0),
                    _cat([fam(0, 72), jnp.zeros((56, 128), _F32)], axis=0),
                )
                for j in range(3):
                    dst[j, pl.ds(c0, 128), :] = tiles[j].T

        def b_qkv(c):
            r0 = pl.multiple_of(c * RC, RC)
            x = xb_v[pl.ds(r0, RC), :]
            zero = jnp.zeros((SB, 128), _BF16)
            k = _dot(x, wqkv_v[:, QW:2 * QW]).astype(_BF16)
            for g in range(NG):
                for u in range(RC // SB):
                    tile = c * (RC // SB) + u
                    kb = k[u * SB:(u + 1) * SB, g * 128:(g + 1) * 128]
                    for h in range(nheads(g)):
                        kp_s[g, tile, h * SB:(h + 1) * SB, :] = jnp.where(
                            masks[h], kb, zero)
            v = _dot(x, wqkv_v[:, 2 * QW:3 * QW])
            lane_q = lax.broadcasted_iota(jnp.int32, (RC, QW), 1) % 128
            v = jnp.where(lane_q >= HPG * DH, 1.0, v).astype(_BF16)
            for g in range(NG):
                for u in range(RC // SB):
                    tile = c * (RC // SB) + u
                    vb = v[u * SB:(u + 1) * SB, g * 128:(g + 1) * 128]
                    for h in range(nheads(g)):
                        vp_s[g, tile, h * SB:(h + 1) * SB, :] = jnp.where(
                            masks[h] | (lane == HPG * DH + h), vb, zero)
            q_s[pl.ds(r0, RC), :] = _dot(x, wqkv_v[:, 0:QW]).astype(_BF16)

        cp["fm"].wait()
        cp["fm0"].wait()

        with jax.named_scope("a_dft"):
            def step(c):
                chunk_copy(xa_h, xa_v, xa_sems, c).wait()
                a_dft(c)
            loop(NRC // 2, step)
            start_rest()
            loop(NRC, step, lo=NRC // 2)

        with jax.named_scope("a_fft16"):
            loop(N2 // 8, lambda r: fft_rows(r, -1.0))

        with jax.named_scope("b_regroup"):
            cp["wqkv"].wait()
            for j in range(3):
                for g in range(NG):
                    n = nheads(g) * DH
                    c0 = j * D + g * HPG * DH
                    blk = wqkv_r[:, c0:c0 + n]
                    wqkv_v[:, j * QW + g * 128:j * QW + (g + 1) * 128] = _cat(
                        [blk, jnp.zeros((D, 128 - n), _BF16)])

        cp["wrt"].wait()
        cp["wit"].wait()

        with jax.named_scope("b_qkv"):
            def step(c):
                chunk_copy(xb_h, xb_v, xb_sems, c).wait()
                b_qkv(c)
                w_prep(2 * c, 0)
                w_prep(2 * c + 1, 1)
            loop(NRC, step)

    pl.run_scoped(
        early,
        pltpu.VMEM((S, D), _BF16),
        pltpu.VMEM((DF, S), _BF16),
        pltpu.VMEM((DF, S), _BF16),
        pltpu.VMEM((S, D), _BF16),
        pltpu.VMEM((D, 3 * D), _BF16),
        pltpu.VMEM((D, 3 * QW), _BF16),
        pltpu.VMEM((4, WTR, 128), _F32),
    )

    def a_mid1(k1, slot):
        r0 = pl.multiple_of(k1 * N2, N2)
        a = zs[pl.ds(r0, N2), :].astype(_BF16)
        pq = _dot(tf_v[k1], a)
        xm_buf[slot, :, 0:FP] = pq[:N2, :FP] - pq[N2:, FP:]
        xm_buf[slot, :, FP:2 * FP] = pq[:N2, FP:] + pq[N2:, :FP]

    def a_mid2(k1, slot):
        xr = xm_buf[slot, :, 0:FP]
        xi = xm_buf[slot, :, FP:2 * FP]
        wr = _cat([wrf[t, pl.ds(k1, N2, stride=N1), :] for t in range(3)])
        wi = _cat([wif[t, pl.ds(k1, N2, stride=N1), :] for t in range(3)])
        ym_buf[slot, :, 0:FP] = (xr * wr - xi * wi).astype(_BF16)
        ym_buf[slot, :, FP:2 * FP] = (xr * wi + xi * wr).astype(_BF16)

    def a_mid3(k1, slot):
        r0 = pl.multiple_of(k1 * N2, N2)
        pq = _dot(tb_v[k1], ym_buf[slot])
        zs[pl.ds(r0, N2), pl.ds(0, FP)] = pq[:N2, :FP] + pq[N2:, FP:]
        zs[pl.ds(r0, N2), pl.ds(FP, FP)] = pq[:N2, FP:] - pq[N2:, :FP]

    late_copy("tf").wait()
    late_copy("tb").wait()

    with jax.named_scope("a_mid"):
        a_mid1(0, 0)
        a_mid1(1, 1)
        a_mid2(0, 0)

        def step(j):
            k = 2 * j
            a_mid1(k + 2, 0)
            a_mid2(k + 1, 1)
            a_mid3(k, 0)
            a_mid1(k + 3, 1)
            a_mid2(k + 2, 0)
            a_mid3(k + 1, 1)

        loop(N1 // 2 - 1, step)
        a_mid2(N1 - 1, 1)
        a_mid3(N1 - 2, 0)
        a_mid3(N1 - 1, 1)

    def attention(s_buf, p_buf):
        row = lax.broadcasted_iota(jnp.int32, (SB, 128), 0)
        col = lax.broadcasted_iota(jnp.int32, (SB, 128), 1) % SB
        bias_diag = jnp.where(col <= row, 0.0, NEG).astype(_F32)
        bias_far = jnp.where(col > row, 0.0, NEG).astype(_F32)
        low = lane < SB

        o_acc[0:(NT - 1) * SB, :] = jnp.zeros(((NT - 1) * SB, QW), _F32)
        for b in range(NT - 1):
            for g in range(NG):
                s_buf[g, b, :, 0:(NT - 1 - b) * GW] = jnp.full(
                    (SB, (NT - 1 - b) * GW), NEG, _F32)

        def b_qk(c, e):
            r0 = pl.multiple_of(c * SB, SB)
            for g in range(NG):
                w = nheads(g) * SB
                out = lax.dot_general(
                    q_s[pl.ds(r0, NT * SB), g * 128:(g + 1) * 128],
                    kp_s[g, c, 0:w, :],
                    (((1,), (1,)), ((), ())), preferred_element_type=_F32)
                for u in range(NT):
                    piece = out[u * SB:(u + 1) * SB, :]
                    if u == 0:
                        piece = piece + _cat([bias_diag] * (w // 128))
                    elif u == NT - 1:
                        piece = piece + _cat([bias_far] * (w // 128))
                    t = NT - 1 - u
                    s_buf[g, (e + u) % RING, :, t * GW:t * GW + w] = piece

        def b_sm(e):
            sl = e % RING
            hb = SB // 2
            for g in range(NG):
                for lp in range(nheads(g) // 2):
                    for rh in range(2):
                        rows = slice(rh * hb, (rh + 1) * hb)
                        xs = [s_buf[g, sl, rows,
                                    t * GW + lp * 128:t * GW + (lp + 1) * 128]
                              for t in range(NT)]
                        mx = xs[0]
                        for t in range(1, NT):
                            mx = jnp.maximum(mx, xs[t])
                        m1 = jnp.max(jnp.where(low, mx, NEG), axis=-1, keepdims=True)
                        m2 = jnp.max(jnp.where(low, NEG, mx), axis=-1, keepdims=True)
                        m = jnp.where(low, m1, m2)
                        for t in range(NT):
                            p_buf[g, sl, rows,
                                  t * GW + lp * 128:t * GW + (lp + 1) * 128] = (
                                jnp.exp2((xs[t] - m) * cexp).astype(_BF16))

        def normalize(o, nh):
            dvalid = (lane >= HPG * DH) & (lane < HPG * DH + nh)
            den = jnp.where(dvalid, o, 1.0)
            r = pl.reciprocal(den, approx=True)
            r = r * (2.0 - den * r)
            r = r * (2.0 - den * r)
            sc = jnp.broadcast_to(r[:, HPG * DH:HPG * DH + 1], o.shape)
            for h in range(1, nh):
                sc = jnp.where(
                    masks[h],
                    jnp.broadcast_to(r[:, HPG * DH + h:HPG * DH + h + 1], o.shape),
                    sc)
            return (o * sc).astype(_BF16)

        def b_pv(c, e):
            r0 = pl.multiple_of(c * SB, SB)
            for g in range(NG):
                w = nheads(g) * SB
                cols = slice(g * 128, (g + 1) * 128)
                lhs = _cat(
                    [p_buf[g, (e + u) % RING, :,
                           (NT - 1 - u) * GW:(NT - 1 - u) * GW + w]
                     for u in range(NT)], axis=0)
                out = _dot(lhs, vp_s[g, c, 0:w, :])
                o_s[pl.ds(r0, SB), cols] = normalize(
                    o_acc[pl.ds(r0, SB), cols] + out[0:SB], nheads(g))
                o_acc[pl.ds(r0 + SB, (NT - 2) * SB), cols] += out[SB:(NT - 1) * SB]
                o_acc[pl.ds(r0 + (NT - 1) * SB, SB), cols] = out[(NT - 1) * SB:]

        nsb = S // SB
        nj = nsb // RING

        def ring_pass(j, first, last):
            for e in range(RING):
                c = RING * j + e
                if not (last and e == RING - 1):
                    b_qk(c + 1, e + 1)
                b_sm(e)
                if not (first and e < NT):
                    b_pv(c - NT, e - NT)

        b_qk(0, 0)
        ring_pass(0, True, False)
        loop(nj - 1, lambda j: ring_pass(j, False, False), lo=1)
        ring_pass(nj - 1, False, True)
        for c in range(nsb - NT, nsb):
            b_pv(c, c)

    with jax.named_scope("b_attn"):
        pl.run_scoped(
            attention,
            pltpu.VMEM((NG, RING, SB, NT * GW), _F32),
            pltpu.VMEM((NG, RING, SB, NT * GW), _BF16),
        )

    def b_out_copy(c):
        r0 = pl.multiple_of(c * RC, RC)
        return pltpu.make_async_copy(
            yb_buf.at[pl.ds(r0, RC), :],
            out_h.at[pl.ds(r0, RC), pl.ds(D, D)],
            ob_sems.at[c])

    def b_proj(c):
        r0 = pl.multiple_of(c * RC, RC)
        yb_buf[pl.ds(r0, RC), :] = _dot(o_s[pl.ds(r0, RC), :], wo_v[...]).astype(_BF16)
        b_out_copy(c).start()

    def a_out_copy(c):
        r0 = pl.multiple_of(c * RC, RC)
        return pltpu.make_async_copy(
            ya_buf.at[pl.ds(r0, RC), :],
            out_h.at[pl.ds(r0, RC), pl.ds(0, D)],
            oa_sems.at[c])

    def a_idft(c):
        r0 = pl.multiple_of(c * RC, RC)
        rows = pl.ds(r0, RC)
        zz = [_cat([zs[rows, t * 128:(t + 1) * 128],
                    zs[rows, FP + t * 128:FP + (t + 1) * 128]]).astype(_BF16)
              for t in range(3)]
        e1 = _dot(zz[0], im_v[0])
        e2 = _dot(zz[1], im_v[1])
        e0 = _dot(zz[2], im0_v[...])
        e1r, e1i = e1[:, :128], e1[:, 128:]
        e2r, e2i = e2[:, :128], e2[:, 128:]
        u1 = e0 + _C1 * e1r + _C2 * e2r
        v1 = _S1 * e1i + _S2 * e2i
        u2 = e0 + _C2 * e1r + _C1 * e2r
        v2 = _S2 * e1i - _S1 * e2i
        ys = (e0 + e1r + e2r, u1 - v1, u2 - v2, u2 + v2, u1 + v1)
        for a in range(5):
            ya_buf[rows, a * 128:(a + 1) * 128] = ys[a].astype(_BF16)
        a_out_copy(c).start()

    for g in range(NG):
        wo_copy(g).wait()

    with jax.named_scope("b_proj"):
        def step(c):
            b_proj(c)
            fft_rows(2 * c, 1.0)
            fft_rows(2 * c + 1, 1.0)
        loop(NRC, step)

    late_copy("im").wait()
    late_copy("im0").wait()

    with jax.named_scope("a_idft"):
        loop(NRC, a_idft)

    for c in range(NRC):
        a_out_copy(c).wait()
        b_out_copy(c).wait()


@jax.jit
def pallas_concat_heads__spectral_gfnet__sliding_block__prompt_kernel(
    A_x: jax.Array,
    A_w_r: jax.Array,
    A_w_i: jax.Array,
    B_x: jax.Array,
    B_wqkv: jax.Array,
    B_wo: jax.Array,
):
    fm, fm0, im, im0, tf, tb = _tables()
    xa = A_x.reshape(S, D)
    xb = B_x.reshape(S, D)

    hbm = pl.BlockSpec(memory_space=pltpu.HBM)
    out = pl.pallas_call(
        _kernel,
        out_shape=jax.ShapeDtypeStruct((S, 2 * D), _BF16),
        in_specs=[hbm] * 12,
        out_specs=hbm,
        scratch_shapes=[
            pltpu.VMEM((QW, D), _BF16),
            pltpu.VMEM((2, 256, 256), _BF16),
            pltpu.VMEM((128, 256), _BF16),
            pltpu.VMEM((2, 256, 256), _BF16),
            pltpu.VMEM((256, 128), _BF16),
            pltpu.VMEM((N1, 2 * N2, N2), _BF16),
            pltpu.VMEM((N1, 2 * N2, N2), _BF16),
            pltpu.VMEM((3, S, 128), _F32),
            pltpu.VMEM((3, S, 128), _F32),
            pltpu.VMEM((S, 2 * FP), _F32),
            pltpu.VMEM((S + 4 * SB, QW), _BF16),
            pltpu.VMEM((NG, S // SB, GW, 128), _BF16),
            pltpu.VMEM((NG, S // SB, GW, 128), _BF16),
            pltpu.VMEM((S + 4 * SB, QW), _F32),
            pltpu.VMEM((S, QW), _BF16),
            pltpu.VMEM((2, N2, 2 * FP), _F32),
            pltpu.VMEM((2, N2, 2 * FP), _BF16),
            pltpu.VMEM((S, D), _BF16),
            pltpu.VMEM((S, D), _BF16),
            pltpu.SemaphoreType.DMA((9,)),
            pltpu.SemaphoreType.DMA((NRC,)),
            pltpu.SemaphoreType.DMA((NRC,)),
            pltpu.SemaphoreType.DMA((NG,)),
            pltpu.SemaphoreType.DMA((NRC,)),
            pltpu.SemaphoreType.DMA((NRC,)),
        ],
        compiler_params=pltpu.CompilerParams(
            vmem_limit_bytes=110 * 1024 * 1024),
    )(xa, A_w_r.T, A_w_i.T, xb, B_wqkv, B_wo, fm, fm0, im, im0, tf, tb)
    return out.reshape(1, S, 2 * D)
```

```python
import math

import numpy as np
import jax
import jax.numpy as jnp
from jax import lax
import jax.experimental.pallas as pl
import jax.experimental.pallas.tpu as pltpu

S = 2048
D = 640
DF = D // 2 + 1
FP = 384
H = 32
DH = 20
WIN = 256
HPG = 6
NG = 6
QW = NG * 128
N1 = 16
N2 = 128
SB = 64
NT = WIN // SB + 1
GW = HPG * SB
OP = NT * SB
RING = 8
RC = 256
NRC = S // RC
WTR = 360
NEG = -1e30

_F32 = jnp.float32
_BF16 = jnp.bfloat16

_C1 = math.cos(2.0 * math.pi / 5.0)
_C2 = math.cos(4.0 * math.pi / 5.0)
_S1 = math.sin(2.0 * math.pi / 5.0)
_S2 = math.sin(4.0 * math.pi / 5.0)


def _tables():
    b = np.arange(128, dtype=np.float64)[:, None]

    def ang(f1, n=64):
        f = f1 + 5.0 * np.arange(n, dtype=np.float64)[None, :]
        return 2.0 * np.pi * ((b * f) % D) / D

    scale = 1.0 / (D * S)
    fm = np.zeros((2, 256, 256), np.float64)
    im = np.zeros((2, 256, 256), np.float64)
    for p, (fa, fb) in enumerate(((1, 4), (2, 3))):
        ta, tb_ = ang(fa), ang(fb)
        fm[p, :128, 0:64] = np.cos(ta)
        fm[p, 128:, 0:64] = np.sin(ta)
        fm[p, :128, 64:128] = np.cos(tb_)
        fm[p, 128:, 64:128] = -np.sin(tb_)
        fm[p, :128, 128:192] = -np.sin(ta)
        fm[p, 128:, 128:192] = np.cos(ta)
        fm[p, :128, 192:256] = -np.sin(tb_)
        fm[p, 128:, 192:256] = -np.cos(tb_)
        c = 2.0 * scale
        im[p, 0:64, :128] = c * np.cos(ta).T
        im[p, 128:192, :128] = -c * np.sin(ta).T
        im[p, 0:64, 128:] = c * np.sin(ta).T
        im[p, 128:192, 128:] = c * np.cos(ta).T
        im[p, 64:128, :128] = c * np.cos(tb_).T
        im[p, 192:256, :128] = -c * np.sin(tb_).T
        im[p, 64:128, 128:] = -c * np.sin(tb_).T
        im[p, 192:256, 128:] = -c * np.cos(tb_).T
    t0 = ang(0, 65)
    fm0 = np.zeros((128, 256), np.float64)
    fm0[:, 0:65] = np.cos(t0)
    fm0[:, 128:128 + 65] = -np.sin(t0)
    cf = np.full((65,), 2.0)
    cf[0] = 1.0
    cf[-1] = 1.0
    im0 = np.zeros((256, 128), np.float64)
    im0[0:65, :] = scale * cf[:, None] * np.cos(t0).T
    im0[128:128 + 65, :] = -scale * cf[:, None] * np.sin(t0).T
    k1 = np.arange(N1)[:, None, None]
    k2 = np.arange(N2)[None, :, None]
    n2 = np.arange(N2)[None, None, :]
    a = 2.0 * np.pi * ((n2 * (k1 + N1 * k2)) % S) / S
    tr = np.cos(a)
    ti = -np.sin(a)
    tf = np.concatenate([tr, ti], axis=1)
    tb = np.concatenate([tr.transpose(0, 2, 1), ti.transpose(0, 2, 1)], axis=1)
    c = lambda t: jnp.asarray(t, _BF16)
    return c(fm), c(fm0), c(im), c(im0), c(tf), c(tb)


def _cmul_const(xr, xi, wr, wi):
    eps = 1e-12
    if abs(wi) < eps:
        if abs(wr - 1.0) < eps:
            return xr, xi
        if abs(wr + 1.0) < eps:
            return -xr, -xi
    if abs(wr) < eps:
        if abs(wi - 1.0) < eps:
            return -xi, xr
        if abs(wi + 1.0) < eps:
            return xi, -xr
    if abs(abs(wr) - abs(wi)) < eps:
        s = abs(wr)
        a = xr * s
        b = xi * s
        sr = 1.0 if wr > 0 else -1.0
        si = 1.0 if wi > 0 else -1.0
        re = (a - b) if (sr > 0 and si > 0) else (a + b) if (sr > 0) else (
            (-a - b) if si > 0 else (b - a))
        im = (a + b) if (si > 0 and sr > 0) else (b - a) if (sr > 0) else (
            (a - b) if si > 0 else (-a - b))
        return re, im
    return xr * wr - xi * wi, xr * wi + xi * wr


def _fft_list(xs, sign):
    n = len(xs)
    if n == 1:
        return xs
    ev = _fft_list(xs[0::2], sign)
    od = _fft_list(xs[1::2], sign)
    out = [None] * n
    for k in range(n // 2):
        ang = sign * 2.0 * math.pi * k / n
        tr, ti = _cmul_const(od[k][0], od[k][1], math.cos(ang), math.sin(ang))
        out[k] = (ev[k][0] + tr, ev[k][1] + ti)
        out[k + n // 2] = (ev[k][0] - tr, ev[k][1] - ti)
    return out


def _dot(a, b):
    return jnp.dot(a, b, preferred_element_type=_F32)


def _cat(xs, axis=1):
    return jnp.concatenate(xs, axis=axis)


def _kernel(xa_h, wrt_h, wit_h, xb_h, wqkv_h, wo_h,
            fm_h, fm0_h, im_h, im0_h, tf_h, tb_h,
            out_h,
            wo_v, fm_v, fm0_v, im_v, im0_v, tf_v, tb_v,
            zs_b, q_s, kp_s, vp_s, o_acc, o_s,
            ya_buf, yb_buf,
            in_sems, xa_sems, xb_sems, wo_sems, oa_sems, ob_sems):
    lane = lax.broadcasted_iota(jnp.int32, (1, 128), 1)
    masks = [((lane >= h * DH) & (lane < (h + 1) * DH)) for h in range(HPG)]
    cexp = (DH ** -0.5) * math.log2(math.e)

    def loop(n, fn, lo=0):
        def body(i, carry):
            fn(i)
            return carry
        lax.fori_loop(lo, n, body, 0)

    def nheads(g):
        return min(HPG, H - g * HPG)

    cp = {}

    def start(idx, name, src, dst):
        cp[name] = pltpu.make_async_copy(src, dst, in_sems.at[idx])
        cp[name].start()

    def late_copy(name):
        idx, src, dst = {"tf": (5, tf_h, tf_v), "tb": (6, tb_h, tb_v),
                         "im": (7, im_h, im_v), "im0": (8, im0_h, im0_v)}[name]
        return pltpu.make_async_copy(src, dst, in_sems.at[idx])

    def wo_copy(g):
        n = nheads(g) * DH
        return pltpu.make_async_copy(
            wo_h.at[pl.ds(g * HPG * DH, n), :],
            wo_v.at[pl.ds(g * 128, n), :], wo_sems.at[g])

    def fft_rows(r, sign, zs):
        r0 = pl.multiple_of(r * 8, 8)
        for t in range(FP // 128):
            xs = []
            for n1 in range(N1):
                rows = pl.ds(n1 * N2 + r0, 8)
                xs.append((zs[rows, pl.ds(t * 128, 128)],
                           zs[rows, pl.ds(FP + t * 128, 128)]))
            ys = _fft_list(xs, sign)
            for k1 in range(N1):
                rows = pl.ds(k1 * N2 + r0, 8)
                zs[rows, pl.ds(t * 128, 128)] = ys[k1][0]
                zs[rows, pl.ds(FP + t * 128, 128)] = ys[k1][1]

    def spectral_and_qkv(wrf, wif, zs_f, xm_buf, ym_buf):
        def early(xa_v, wrt_v, wit_v, xb_v, wqkv_r, wqkv_v, wtf):
            def chunk_copy(src, dst, sems, c):
                r0 = pl.multiple_of(c * RC, RC)
                return pltpu.make_async_copy(
                    src.at[pl.ds(r0, RC), :], dst.at[pl.ds(r0, RC), :], sems.at[c])

            start(0, "fm", fm_h, fm_v)
            start(1, "fm0", fm0_h, fm0_v)
            for c in range(4):
                chunk_copy(xa_h, xa_v, xa_sems, c).start()

            for g in range(NG):
                n = nheads(g) * DH
                wo_v[g * 128 + n:(g + 1) * 128, :] = jnp.zeros((128 - n, D), _BF16)

            def start_rest():
                for c in range(1, 3):
                    chunk_copy(xb_h, xb_v, xb_sems, c).start()
                start(3, "wrt", wrt_h, wrt_v)
                start(4, "wit", wit_h, wit_v)
                for c in range(3, NRC):
                    chunk_copy(xb_h, xb_v, xb_sems, c).start()
                late_copy("tf").start()
                late_copy("tb").start()
                for g in range(NG):
                    wo_copy(g).start()
                late_copy("im").start()
                late_copy("im0").start()

            for b in range(4):
                wtf[b, 320:WTR, :] = jnp.zeros((WTR - 320, 128), _F32)
            q_s[S:S + 4 * SB, :] = jnp.zeros((4 * SB, QW), _BF16)

            def a_dft(c):
                r0 = pl.multiple_of(c * RC, RC)
                rows = pl.ds(r0, RC)
                xs = [xa_v[rows, a * 128:(a + 1) * 128].astype(_F32) for a in range(5)]
                t1 = xs[1] + xs[4]
                t2 = xs[2] + xs[3]
                t3 = xs[1] - xs[4]
                t4 = xs[2] - xs[3]
                a0 = xs[0] + t1 + t2
                a1r = xs[0] + _C1 * t1 + _C2 * t2
                a1i = -(_S1 * t3 + _S2 * t4)
                a2r = xs[0] + _C2 * t1 + _C1 * t2
                a2i = _S1 * t4 - _S2 * t3
                m1 = _dot(_cat([a1r, a1i]).astype(_BF16), fm_v[0])
                m2 = _dot(_cat([a2r, a2i]).astype(_BF16), fm_v[1])
                m0 = _dot(a0.astype(_BF16), fm0_v[...])
                for t, m in enumerate((m1, m2, m0)):
                    zs_f[rows, t * 128:(t + 1) * 128] = m[:, :128]
                    zs_f[rows, FP + t * 128:FP + (t + 1) * 128] = m[:, 128:]

            def w_prep(t, slot):
                c0 = pl.multiple_of(t * 128, 128)
                for b, (src, dst) in enumerate(((wrt_v, wrf), (wit_v, wif))):
                    stage = wtf.at[2 * slot + b]
                    stage[0:DF, :] = src[:, pl.ds(c0, 128)].astype(_F32)
                    fam = lambda f1, n: stage[pl.ds(f1, n, stride=5), :]
                    tiles = (
                        _cat([fam(1, 64), fam(4, 64)], axis=0),
                        _cat([fam(2, 64), fam(3, 64)], axis=0),
                        _cat([fam(0, 72), jnp.zeros((56, 128), _F32)], axis=0),
                    )
                    for j in range(3):
                        dst[j, pl.ds(c0, 128), :] = tiles[j].T

            def b_qkv(c):
                r0 = pl.multiple_of(c * RC, RC)
                x = xb_v[pl.ds(r0, RC), :]
                zero = jnp.zeros((SB, 128), _BF16)
                k = _dot(x, wqkv_v[:, QW:2 * QW]).astype(_BF16)
                for g in range(NG):
                    for u in range(RC // SB):
                        tile = c * (RC // SB) + u
                        kb = k[u * SB:(u + 1) * SB, g * 128:(g + 1) * 128]
                        for h in range(nheads(g)):
                            kp_s[g, tile, h * SB:(h + 1) * SB, :] = jnp.where(
                                masks[h], kb, zero)
                v = _dot(x, wqkv_v[:, 2 * QW:3 * QW])
                lane_q = lax.broadcasted_iota(jnp.int32, (RC, QW), 1) % 128
                v = jnp.where(lane_q >= HPG * DH, 1.0, v).astype(_BF16)
                for g in range(NG):
                    for u in range(RC // SB):
                        tile = c * (RC // SB) + u
                        vb = v[u * SB:(u + 1) * SB, g * 128:(g + 1) * 128]
                        for h in range(nheads(g)):
                            vp_s[g, tile, h * SB:(h + 1) * SB, :] = jnp.where(
                                masks[h] | (lane == HPG * DH + h), vb, zero)
                q_s[pl.ds(r0, RC), :] = _dot(x, wqkv_v[:, 0:QW]).astype(_BF16)

            with jax.named_scope("wait_fm"):
                cp["fm"].wait()
                cp["fm0"].wait()

            with jax.named_scope("a_dft"):
                def step_pf(c):
                    chunk_copy(xa_h, xa_v, xa_sems, c).wait()
                    chunk_copy(xa_h, xa_v, xa_sems, c + 4).start()
                    a_dft(c)

                def step(c):
                    chunk_copy(xa_h, xa_v, xa_sems, c).wait()
                    a_dft(c)

                loop(4, step_pf)
                start(2, "wqkv", wqkv_h, wqkv_r)
                loop(NRC - 1, step, lo=4)
                chunk_copy(xb_h, xb_v, xb_sems, 0).start()
                loop(NRC, step, lo=NRC - 1)

            with jax.named_scope("a_fft16"):
                loop(N2 // 8, lambda r: fft_rows(r, -1.0, zs_f))

            with jax.named_scope("b_regroup"):
                cp["wqkv"].wait()
                start_rest()
                for j in range(3):
                    for g in range(NG):
                        n = nheads(g) * DH
                        c0 = j * D + g * HPG * DH
                        blk = wqkv_r[:, c0:c0 + n]
                        wqkv_v[:, j * QW + g * 128:j * QW + (g + 1) * 128] = _cat(
                            [blk, jnp.zeros((D, 128 - n), _BF16)])

            with jax.named_scope("b_qkv"):
                def step0(c):
                    chunk_copy(xb_h, xb_v, xb_sems, c).wait()
                    b_qkv(c)

                def step1(c):
                    chunk_copy(xb_h, xb_v, xb_sems, c).wait()
                    b_qkv(c)
                    for u in range(4):
                        w_prep(4 * (c - NRC // 2) + u, u % 2)

                loop(NRC // 2, step0)
                cp["wrt"].wait()
                cp["wit"].wait()
                loop(NRC, step1, lo=NRC // 2)

        pl.run_scoped(
            early,
            pltpu.VMEM((S, D), _BF16),
            pltpu.VMEM((DF, S), _BF16),
            pltpu.VMEM((DF, S), _BF16),
            pltpu.VMEM((S, D), _BF16),
            pltpu.VMEM((D, 3 * D), _BF16),
            pltpu.VMEM((D, 3 * QW), _BF16),
            pltpu.VMEM((4, WTR, 128), _F32),
        )

        def a_mid1(k1, slot):
            r0 = pl.multiple_of(k1 * N2, N2)
            a = zs_f[pl.ds(r0, N2), :].astype(_BF16)
            pq = _dot(tf_v[k1], a)
            xm_buf[slot, :, 0:FP] = pq[:N2, :FP] - pq[N2:, FP:]
            xm_buf[slot, :, FP:2 * FP] = pq[:N2, FP:] + pq[N2:, :FP]

        def a_mid2(k1, slot):
            xr = xm_buf[slot, :, 0:FP]
            xi = xm_buf[slot, :, FP:2 * FP]
            wr = _cat([wrf[t, pl.ds(k1, N2, stride=N1), :] for t in range(3)])
            wi = _cat([wif[t, pl.ds(k1, N2, stride=N1), :] for t in range(3)])
            ym_buf[slot, :, 0:FP] = (xr * wr - xi * wi).astype(_BF16)
            ym_buf[slot, :, FP:2 * FP] = (xr * wi + xi * wr).astype(_BF16)

        def a_mid3(k1, slot):
            r0 = pl.multiple_of(k1 * N2, N2)
            pq = _dot(tb_v[k1], ym_buf[slot])
            zs_b[pl.ds(r0, N2), pl.ds(0, FP)] = pq[:N2, :FP] + pq[N2:, FP:]
            zs_b[pl.ds(r0, N2), pl.ds(FP, FP)] = pq[:N2, FP:] - pq[N2:, :FP]

        late_copy("tf").wait()
        late_copy("tb").wait()

        with jax.named_scope("a_mid"):
            a_mid1(0, 0)
            a_mid1(1, 1)
            a_mid2(0, 0)

            def step(j):
                k = 2 * j
                a_mid1(k + 2, 0)
                a_mid2(k + 1, 1)
                a_mid3(k, 0)
                a_mid1(k + 3, 1)
                a_mid2(k + 2, 0)
                a_mid3(k + 1, 1)

            loop(N1 // 2 - 1, step)
            a_mid2(N1 - 1, 1)
            a_mid3(N1 - 2, 0)
            a_mid3(N1 - 1, 1)

    pl.run_scoped(
        spectral_and_qkv,
        pltpu.VMEM((3, S, 128), _F32),
        pltpu.VMEM((3, S, 128), _F32),
        pltpu.VMEM((S, 2 * FP), _F32),
        pltpu.VMEM((2, N2, 2 * FP), _F32),
        pltpu.VMEM((2, N2, 2 * FP), _BF16),
    )

    def attention(s_buf, p_buf):
        row = lax.broadcasted_iota(jnp.int32, (SB, 128), 0)
        col = lax.broadcasted_iota(jnp.int32, (SB, 128), 1) % SB
        bias_diag = jnp.where(col <= row, 0.0, NEG).astype(_F32)
        bias_far = jnp.where(col > row, 0.0, NEG).astype(_F32)
        low = lane < SB

        o_acc[OP:OP + (NT - 1) * SB, :] = jnp.zeros(((NT - 1) * SB, QW), _F32)
        for b in range(NT - 1):
            for g in range(NG):
                s_buf[g, b, :, 0:(NT - 1 - b) * GW] = jnp.full(
                    (SB, (NT - 1 - b) * GW), NEG, _F32)

        def b_qk(c, e):
            r0 = pl.multiple_of(c * SB, SB)
            for g in range(NG):
                w = nheads(g) * SB
                out = lax.dot_general(
                    q_s[pl.ds(r0, NT * SB), g * 128:(g + 1) * 128],
                    kp_s[g, c, 0:w, :],
                    (((1,), (1,)), ((), ())), preferred_element_type=_F32)
                for u in range(NT):
                    piece = out[u * SB:(u + 1) * SB, :]
                    if u == 0:
                        piece = piece + _cat([bias_diag] * (w // 128))
                    elif u == NT - 1:
                        piece = piece + _cat([bias_far] * (w // 128))
                    t = NT - 1 - u
                    s_buf[g, (e + u) % RING, :, t * GW:t * GW + w] = piece

        def b_sm(e):
            sl = e % RING
            hb = SB // 2
            for g in range(NG):
                for lp in range(nheads(g) // 2):
                    for rh in range(2):
                        rows = slice(rh * hb, (rh + 1) * hb)
                        xs = [s_buf[g, sl, rows,
                                    t * GW + lp * 128:t * GW + (lp + 1) * 128]
                              for t in range(NT)]
                        mx = xs[0]
                        for t in range(1, NT):
                            mx = jnp.maximum(mx, xs[t])
                        m1 = jnp.max(jnp.where(low, mx, NEG), axis=-1, keepdims=True)
                        m2 = jnp.max(jnp.where(low, NEG, mx), axis=-1, keepdims=True)
                        m = jnp.where(low, m1, m2)
                        for t in range(NT):
                            p_buf[g, sl, rows,
                                  t * GW + lp * 128:t * GW + (lp + 1) * 128] = (
                                jnp.exp2((xs[t] - m) * cexp).astype(_BF16))

        def normalize(o, nh):
            dvalid = (lane >= HPG * DH) & (lane < HPG * DH + nh)
            den = jnp.where(dvalid, o, 1.0)
            r = pl.reciprocal(den, approx=True)
            r = r * (2.0 - den * r)
            r = r * (2.0 - den * r)
            sc = jnp.broadcast_to(r[:, HPG * DH:HPG * DH + 1], o.shape)
            for h in range(1, nh):
                sc = jnp.where(
                    masks[h],
                    jnp.broadcast_to(r[:, HPG * DH + h:HPG * DH + h + 1], o.shape),
                    sc)
            return (o * sc).astype(_BF16)

        def b_pv(c, e):
            r0 = pl.multiple_of(c * SB + OP, SB)
            for g in range(NG):
                w = nheads(g) * SB
                cols = slice(g * 128, (g + 1) * 128)
                lhs = _cat(
                    [p_buf[g, (e + u) % RING, :,
                           (NT - 1 - u) * GW:(NT - 1 - u) * GW + w]
                     for u in range(NT)], axis=0)
                out = _dot(lhs, vp_s[g, c, 0:w, :])
                o_s[pl.ds(r0, SB), cols] = normalize(
                    o_acc[pl.ds(r0, SB), cols] + out[0:SB], nheads(g))
                o_acc[pl.ds(r0 + SB, (NT - 2) * SB), cols] += out[SB:(NT - 1) * SB]
                o_acc[pl.ds(r0 + (NT - 1) * SB, SB), cols] = out[(NT - 1) * SB:]

        nsb = S // SB
        nj = nsb // RING

        def ring_pass(j, first, last):
            for e in range(RING):
                c = RING * j + e
                if not (last and e == RING - 1):
                    b_qk(c + 1, e + 1)
                b_sm(e)
                if not (first and e < NT):
                    b_pv(c - NT, e - NT)
                if e % 2 == 1:
                    fft_rows((RING // 2) * j + e // 2, 1.0, zs_b)

        b_qk(0, 0)
        ring_pass(0, True, False)
        loop(nj - 1, lambda j: ring_pass(j, False, False), lo=1)
        ring_pass(nj - 1, False, True)
        for c in range(nsb - NT, nsb):
            b_pv(c, c)

    with jax.named_scope("b_attn"):
        pl.run_scoped(
            attention,
            pltpu.VMEM((NG, RING, SB, NT * GW), _F32),
            pltpu.VMEM((NG, RING, SB, NT * GW), _BF16),
        )

    def b_out_copy(c):
        r0 = pl.multiple_of(c * RC, RC)
        return pltpu.make_async_copy(
            yb_buf.at[pl.ds(r0, RC), :],
            out_h.at[pl.ds(r0, RC), pl.ds(D, D)],
            ob_sems.at[c])

    def b_proj(c):
        r0 = pl.multiple_of(c * RC, RC)
        yb_buf[pl.ds(r0, RC), :] = _dot(o_s[pl.ds(OP + r0, RC), :], wo_v[...]).astype(_BF16)
        b_out_copy(c).start()

    def a_out_copy(c):
        r0 = pl.multiple_of(c * RC, RC)
        return pltpu.make_async_copy(
            ya_buf.at[pl.ds(r0, RC), :],
            out_h.at[pl.ds(r0, RC), pl.ds(0, D)],
            oa_sems.at[c])

    def a_idft(c):
        r0 = pl.multiple_of(c * RC, RC)
        rows = pl.ds(r0, RC)
        zz = [_cat([zs_b[rows, t * 128:(t + 1) * 128],
                    zs_b[rows, FP + t * 128:FP + (t + 1) * 128]]).astype(_BF16)
              for t in range(3)]
        e1 = _dot(zz[0], im_v[0])
        e2 = _dot(zz[1], im_v[1])
        e0 = _dot(zz[2], im0_v[...])
        e1r, e1i = e1[:, :128], e1[:, 128:]
        e2r, e2i = e2[:, :128], e2[:, 128:]
        u1 = e0 + _C1 * e1r + _C2 * e2r
        v1 = _S1 * e1i + _S2 * e2i
        u2 = e0 + _C2 * e1r + _C1 * e2r
        v2 = _S2 * e1i - _S1 * e2i
        ys = (e0 + e1r + e2r, u1 - v1, u2 - v2, u2 + v2, u1 + v1)
        for a in range(5):
            ya_buf[rows, a * 128:(a + 1) * 128] = ys[a].astype(_BF16)
        a_out_copy(c).start()

    for g in range(NG):
        wo_copy(g).wait()

    late_copy("im").wait()
    late_copy("im0").wait()

    with jax.named_scope("b_proj"):
        def step(c):
            b_proj(c)
            a_idft(c)
        loop(NRC, step)

    for c in range(NRC):
        a_out_copy(c).wait()
        b_out_copy(c).wait()


@jax.jit
def pallas_concat_heads__spectral_gfnet__sliding_block__prompt_kernel(
    A_x: jax.Array,
    A_w_r: jax.Array,
    A_w_i: jax.Array,
    B_x: jax.Array,
    B_wqkv: jax.Array,
    B_wo: jax.Array,
):
    fm, fm0, im, im0, tf, tb = _tables()
    xa = A_x.reshape(S, D)
    xb = B_x.reshape(S, D)

    hbm = pl.BlockSpec(memory_space=pltpu.HBM)
    out = pl.pallas_call(
        _kernel,
        out_shape=jax.ShapeDtypeStruct((S, 2 * D), _BF16),
        in_specs=[hbm] * 12,
        out_specs=hbm,
        scratch_shapes=[
            pltpu.VMEM((QW, D), _BF16),
            pltpu.VMEM((2, 256, 256), _BF16),
            pltpu.VMEM((128, 256), _BF16),
            pltpu.VMEM((2, 256, 256), _BF16),
            pltpu.VMEM((256, 128), _BF16),
            pltpu.VMEM((N1, 2 * N2, N2), _BF16),
            pltpu.VMEM((N1, 2 * N2, N2), _BF16),
            pltpu.VMEM((S, 2 * FP), _F32),
            pltpu.VMEM((S + 4 * SB, QW), _BF16),
            pltpu.VMEM((NG, S // SB, GW, 128), _BF16),
            pltpu.VMEM((NG, S // SB, GW, 128), _BF16),
            pltpu.VMEM((OP + S + 4 * SB, QW), _F32),
            pltpu.VMEM((OP + S, QW), _BF16),
            pltpu.VMEM((S, D), _BF16),
            pltpu.VMEM((S, D), _BF16),
            pltpu.SemaphoreType.DMA((9,)),
            pltpu.SemaphoreType.DMA((NRC,)),
            pltpu.SemaphoreType.DMA((NRC,)),
            pltpu.SemaphoreType.DMA((NG,)),
            pltpu.SemaphoreType.DMA((NRC,)),
            pltpu.SemaphoreType.DMA((NRC,)),
        ],
        compiler_params=pltpu.CompilerParams(
            vmem_limit_bytes=110 * 1024 * 1024),
    )(xa, A_w_r.T, A_w_i.T, xb, B_wqkv, B_wo, fm, fm0, im, im0, tf, tb)
    return out.reshape(1, S, 2 * D)
```
